```python
import os as _os
_os.environ.setdefault("JAX_PLATFORMS", "cpu")
import jax
import jax.numpy as jnp

def _softmax(x, axis=-1):
    return jax.nn.softmax(x, axis=axis)
def _gelu(x):
    return jax.nn.gelu(x, approximate=True)
def _silu(x):
    return jax.nn.silu(x)
def _sigmoid(x):
    return jax.nn.sigmoid(x)
def _layernorm(x, axis=-1, eps=1e-5):
    m = jnp.mean(x, axis=axis, keepdims=True)
    v = jnp.var(x, axis=axis, keepdims=True)
    return (x - m) / jnp.sqrt(v + eps)
def _scatter_add(tgt, idx, src, axis=0):
    return tgt.at[idx].add(src)
def _segment_sum(src, seg, n):
    return jax.ops.segment_sum(src, seg, n)
class _Rng:
    def __init__(self, key):
        self._k = key
    def _next(self):
        self._k, sub = jax.random.split(self._k)
        return sub
    def normal(self, shape):
        return jax.random.normal(self._next(), shape, dtype=jnp.bfloat16)
    def randint(self, lo, hi, shape):
        return jax.random.randint(self._next(), shape, lo, hi, dtype=jnp.int32)
    def uniform(self, shape, lo=0.0, hi=1.0):
        return jax.random.uniform(self._next(), shape, jnp.bfloat16, lo, hi)
    def permutation(self, n):
        return jax.random.permutation(self._next(), n)


kernel_name = 'concat_heads__compressed_kv_cla__gqa_block_cached__decode'

def setup_inputs():
    _rng = _Rng(jax.random.key(int.from_bytes(__import__("os").urandom(4), "little")))
    _w = (lambda a: (lambda t: t.astype(jnp.bfloat16) if jnp.issubdtype(t.dtype, jnp.floating) else t)(jnp.asarray(a)))
    def _A_setup():
        B, H, Sq, Sk, D, M = 4, 32, 1, 4096, 128, 512
        Dc = 4 * D
        return {
            "x": _w((lambda *s: _rng.normal(s) * 3.2)(B, Sq, M)),
            "c_kv": _w((lambda *s: _rng.normal(s) * 0.05)(B, Sk, Dc)),
            "w_q": _w((lambda *s: _rng.normal(s) * 3.2)(M, H, D) * (M ** -0.5)),
            "w_uk": _w((lambda *s: _rng.normal(s) * 3.2)(Dc, H, D) * (Dc ** -0.5)),
            "w_uv": _w((lambda *s: _rng.normal(s) * 0.05)(Dc, H, D) * (Dc ** -0.5)),
            "w_o": _w((lambda *s: _rng.normal(s) * 0.05)(H, D, M) * ((H * D) ** -0.5)),
        }
    _A_in = _A_setup()

    def _B_setup():
        B, Sq, D = 4, 1, 512
        Hq, Hkv, Sk, Dh = 32, 8, 4096, 128
        assert Hq % Hkv == 0, (Hq, Hkv)
        return {
            "x": _w((lambda *s: _rng.normal(s) * 0.8)(B, Sq, D)),
            "k_cache": _w((lambda *s: _rng.normal(s) * 0.8)(B, Hkv, Sk, Dh)),
            "v_cache": _w((lambda *s: _rng.normal(s) * 0.05)(B, Hkv, Sk, Dh)),
            "wq": _w((lambda *s: _rng.normal(s) * 0.8)(D, Hq * Dh) * (D ** -0.5)),
            "wo": _w((lambda *s: _rng.normal(s) * 0.05)(Hq * Dh, D) * ((Hq * Dh) ** -0.5)),
        }
    _B_in = _B_setup()

    return {
        "A_x": _A_in["x"],
        "A_c_kv": _A_in["c_kv"],
        "A_w_q": _A_in["w_q"],
        "A_w_uk": _A_in["w_uk"],
        "A_w_uv": _A_in["w_uv"],
        "A_w_o": _A_in["w_o"],
        "B_x": _B_in["x"],
        "B_k_cache": _B_in["k_cache"],
        "B_v_cache": _B_in["v_cache"],
        "B_wq": _B_in["wq"],
        "B_wo": _B_in["wo"],
    }

def reference(A_x, A_c_kv, A_w_q, A_w_uk, A_w_uv, A_w_o, B_x, B_k_cache, B_v_cache, B_wq, B_wo):
    def _A_ref(x, c_kv, w_q, w_uk, w_uv, w_o):
        B, Sq, M = x.shape[0], x.shape[1], x.shape[2]
        Sk = c_kv.shape[1]
        H, D = w_q.shape[1], w_q.shape[2]
        q = jnp.einsum("bqm,mhd->bhqd", x, w_q)
        k = jnp.einsum("bkc,chd->bhkd", c_kv, w_uk)
        v = jnp.einsum("bkc,chd->bhkd", c_kv, w_uv)
        scores = jnp.einsum("bhqd,bhkd->bhqk", q, k) * (D ** -0.5)
        off = Sk - Sq
        qi = jnp.arange(Sq)[:, None]
        kj = jnp.arange(Sk)[None, :]
        cmask = kj <= (qi + off)
        scores = jnp.where(cmask[None, None], scores, -1e9)
        p = _softmax(scores, axis=-1)
        ctx = jnp.einsum("bhqk,bhkd->bhqd", p, v)
        return jnp.einsum("bhqd,hdm->bqm", ctx, w_o)

    def _B_ref(x, k_cache, v_cache, wq, wo):
        B, Sq, D = x.shape
        Hq, Dh = 32, 128
        Hkv = k_cache.shape[1]
        rep = Hq // Hkv
        q = (lambda x, *d: x.transpose(*d))((x @ wq).reshape(B, Sq, Hq, Dh), 0, 2, 1, 3)
        k = jnp.repeat(k_cache, rep, axis=1)
        v = jnp.repeat(v_cache, rep, axis=1)
        scores = jnp.einsum("bhqd,bhkd->bhqk", q, k) * (Dh ** -0.5)
        p = _softmax(scores, axis=-1)
        o = jnp.einsum("bhqk,bhkd->bhqd", p, v)
        return (lambda x, *d: x.transpose(*d))(o, 0, 2, 1, 3).reshape(B, Sq, Hq * Dh) @ wo

    a = _A_ref(A_x, A_c_kv, A_w_q, A_w_uk, A_w_uv, A_w_o)
    b = _B_ref(B_x, B_k_cache, B_v_cache, B_wq, B_wo)
    return jnp.concatenate([a, b], axis=-1)
```

```python
import jax
import jax.numpy as jnp
from jax import lax
import jax.experimental.pallas as pl
import jax.experimental.pallas.tpu as pltpu

F32 = jnp.float32
BF16 = jnp.bfloat16
NT = (((1,), (1,)), ((), ()))
NN = (((1,), (0,)), ((), ()))

N_GROUPS = 13
UNITS = 8
N_UNITS = N_GROUPS * UNITS
LOOKAHEAD = 4
G_W0, G_W1, G_C0, G_KV0, G_W2 = 0, 1, 2, 4, 12
ORDER8 = (0, 1, 2, 3, 4, 5, 6, 7)


def _dot(a, b, dims):
    return lax.dot_general(a, b, dims, preferred_element_type=F32)


def _fold_lanes(x, op):
    r = x[:, 0:128]
    for t in range(1, x.shape[1] // 128):
        r = op(r, x[:, t * 128:(t + 1) * 128])
    return r


def _kernel(xa_hbm, ckv_hbm, wqa_hbm, wuk_hbm, wuv_hbm, woa_hbm,
            xb_hbm, k_hbm, v_hbm, wqb_hbm, wob_hbm,
            out_ref,
            xa_buf, xb_buf, wqa_raw, wuk_raw, wuv_raw, wqa_t, wuk_t, wuv_t,
            wqb_buf, woa_buf, wob_buf, kbuf, vbuf, cbuf,
            x8_ref, ql_hb, qlat, qb_hb, qb, sb, mb, lb, ob, ob_bh, ob_hb,
            sa, ma, la, acca, cl_hb, ctxa, outacc,
            sems):
    scale = 128.0 ** -0.5

    def piece(kind, j, i):
        if kind == "n128":
            return pl.ds(pl.multiple_of(j * 512 + i * 128, 128), 128), slice(None)
        if kind == "n512":
            return pl.ds(pl.multiple_of(j * 128 + i * 32, 32), 32), slice(None)
        return pl.ds(pl.multiple_of(j * 16, 16), 16), pl.ds(i * 1024, 1024)

    def unit_rows(kind, j):
        n = {"n128": 512, "n512": 128, "wide": 16}[kind]
        return pl.ds(pl.multiple_of(j * n, n), n)

    def start_piece(src, s_src, dst, s_dst, kind, j, i, sem, prio):
        rows, cols = piece(kind, j, i)
        pltpu.make_async_copy(src.at[s_src, rows, cols], dst.at[s_dst, rows, cols],
                              sem).start(priority=prio)

    def start_pair(parts, j):
        for i in range(4):
            for s in range(4):
                for p, (src, dst, kind) in enumerate(parts):
                    start_piece(src, s, dst, s, kind, j, i, sems.at[p, j], p)

    def wait_part(parts, p, j):
        _, dst, kind = parts[p]
        view = dst.at[:, unit_rows(kind, j), :]
        pltpu.make_async_copy(view, view, sems.at[p, j]).wait()

    def start_single(src, sbase, dst, dbase, kind, j):
        for i in range(4):
            for n, s in enumerate(ORDER8):
                start_piece(src, sbase + s, dst, dbase + s, kind, j, i, sems.at[0, j], n % 2)

    def wait_single(dst, dbase, kind, j):
        view = dst.at[pl.ds(dbase, 8), unit_rows(kind, j), :]
        pltpu.make_async_copy(view, view, sems.at[0, j]).wait()

    parts_w0 = ((wqa_hbm, wqa_raw, "n128"), (wuk_hbm, wuk_raw, "n128"))
    parts_w1 = ((wuv_hbm, wuv_raw, "n128"), (wqb_hbm, wqb_buf, "wide"))
    parts_w2 = ((woa_hbm, woa_buf, "n512"), (wob_hbm, wob_buf, "n512"))

    def start_last_unit():
        j = UNITS - 1
        for n in range(16):
            start_piece(woa_hbm, n % 4, woa_buf, n % 4, "n512", j, n // 4, sems.at[0, j], 0)
            start_piece(wob_hbm, n // 4, wob_buf, n // 4, "n512", j, n % 4, sems.at[2, n // 4], 1)

    def dispatch(u, w0, w1, c, k, v, w2):
        g = u // UNITS
        j = u % UNITS
        is_kv = jnp.logical_and(g >= G_KV0, g < G_W2)
        b = jnp.clip((g - G_KV0) // 2, 0, 3)
        pl.when(g == G_W0)(lambda: w0(j))
        pl.when(g == G_W1)(lambda: w1(j))
        pl.when(jnp.logical_and(g >= G_C0, g < G_KV0))(lambda: c(g - G_C0, j))
        pl.when(jnp.logical_and(is_kv, g % 2 == 0))(lambda: k(b, j))
        pl.when(jnp.logical_and(is_kv, g % 2 == 1))(lambda: v(b, j))
        pl.when(jnp.logical_and(g == G_W2, j < UNITS - 1))(lambda: w2(j))

    def issue(u):
        dispatch(
            u,
            lambda j: start_pair(parts_w0, j),
            lambda j: start_pair(parts_w1, j),
            lambda pair, j: start_single(ckv_hbm, pair * 8, cbuf, pair * 8, "n512", j),
            lambda b, j: start_single(k_hbm, b * 8, kbuf, 0, "n128", j),
            lambda b, j: start_single(v_hbm, b * 8, vbuf, 0, "n128", j),
            lambda j: start_pair(parts_w2, j),
        )
        pl.when(u == N_UNITS - 1)(start_last_unit)

    def head_major(raw, dst, j):
        for s in range(4):
            blk = raw[s, unit_rows("n128", j), :].reshape(16, 32, 128)
            d0 = pl.multiple_of(s * 128 + j * 16, 16)
            dst[:, pl.ds(d0, 16), :] = jnp.swapaxes(blk, 0, 1)

    def step_w0(j):
        wait_part(parts_w0, 0, j)
        wait_part(parts_w0, 1, j)
        head_major(wqa_raw, wqa_t, j)
        head_major(wuk_raw, wuk_t, j)

    def step_w1(j):
        wait_part(parts_w1, 0, j)
        wait_part(parts_w1, 1, j)
        head_major(wuv_raw, wuv_t, j)
        xa8 = x8_ref[0].astype(BF16)
        for t in range(4):
            h = j * 4 + t
            q = _dot(xa8, wqa_t[h], NN).astype(BF16)
            ql_hb[h] = _dot(q, wuk_t[h], NT) * scale

    def c_block(b, j):
        return cbuf[pl.ds(b * 4, 4), unit_rows("n512", j), :].reshape(512, 512)

    def step_c(pair, j):
        @pl.when(jnp.logical_and(pair == 0, j == 0))
        def _():
            qlat[...] = jnp.swapaxes(ql_hb[...], 0, 1)[0:4].astype(BF16)
            ma[...] = jnp.full(ma.shape, -jnp.inf, F32)

        @pl.when(pair == 0)
        def _():
            xb8 = x8_ref[1].astype(BF16)
            cols = pl.ds(pl.multiple_of(j * 512, 512), 512)
            qc = _dot(xb8, wqb_buf[:, :, cols].reshape(512, 512), NN)
            for r in range(4):
                qb_hb[j * 4 + r] = qc[:, r * 128:(r + 1) * 128]

        wait_single(cbuf, pair * 8, "n512", j)
        for t in range(2):
            b = pair * 2 + t
            s = _dot(qlat[b], c_block(b, j), NT)
            sa[b, j] = s
            ma[b] = jnp.maximum(ma[b], _fold_lanes(s, jnp.maximum))

    low_rows = lax.broadcasted_iota(jnp.int32, (8, 1), 0) < 4

    def step_k(b, j):
        @pl.when(jnp.logical_and(b == 0, j == 0))
        def _():
            qb[...] = jnp.swapaxes(qb_hb[...], 0, 1)[0:4]
            ob_bh[...] = jnp.zeros(ob_bh.shape, F32)
            m = jnp.max(ma[...], axis=-1, keepdims=True)
            ma[...] = jnp.broadcast_to(m, ma.shape)
            la[...] = jnp.zeros(la.shape, F32)
            acca[...] = jnp.zeros(acca.shape, F32)

        @pl.when(jnp.logical_and(b == 2, j == 0))
        def _():
            l = jnp.sum(la[...], axis=-1, keepdims=True)
            cl = jnp.concatenate([acca[...] / l, jnp.zeros((4, 32, 512), F32)], axis=0)
            cl_hb[...] = jnp.swapaxes(cl, 0, 1)

        @pl.when(j == 0)
        def _():
            mb[...] = jnp.full(mb.shape, -jnp.inf, F32)

        wait_single(kbuf, 0, "n128", j)
        rows = unit_rows("n128", j)
        for t in range(4):
            q8 = qb[b, t * 8:(t + 1) * 8, :].astype(BF16)
            s0 = _dot(q8, kbuf[2 * t, rows, :], NT)
            s1 = _dot(q8, kbuf[2 * t + 1, rows, :], NT)
            s = jnp.where(low_rows, s0, s1) * scale
            sb[j, t * 8:(t + 1) * 8, :] = s
            mb[t * 8:(t + 1) * 8, :] = jnp.maximum(
                mb[t * 8:(t + 1) * 8, :], _fold_lanes(s, jnp.maximum))

    def step_v(b, j):
        @pl.when(j == 0)
        def _():
            m = jnp.max(mb[...], axis=-1, keepdims=True)
            mb[...] = jnp.broadcast_to(m, mb.shape)
            lb[...] = jnp.zeros(lb.shape, F32)
            ob[...] = jnp.zeros(ob.shape, F32)

        @pl.when(b < 2)
        def _():
            for t in range(2):
                ba = b * 2 + t
                p = jnp.exp(sa[ba, j] - jnp.concatenate([ma[ba]] * 4, axis=1))
                la[ba] += _fold_lanes(p, jnp.add)
                acca[ba] += _dot(p.astype(BF16), c_block(ba, j), NN)

        @pl.when(b == 2)
        def _():
            for t in range(4):
                h = j * 4 + t
                ctxa[h] = _dot(cl_hb[h].astype(BF16), wuv_t[h], NN)

        m = mb[...]
        p = jnp.exp(sb[j] - jnp.concatenate([m] * 4, axis=1))
        lb[...] += _fold_lanes(p, jnp.add)
        wait_single(vbuf, 0, "n128", j)
        rows = unit_rows("n128", j)
        for t in range(4):
            p8 = p[t * 8:(t + 1) * 8, :].astype(BF16)
            o0 = _dot(p8, vbuf[2 * t, rows, :], NN)
            o1 = _dot(p8, vbuf[2 * t + 1, rows, :], NN)
            ob[t * 8:(t + 1) * 8, :] += jnp.where(low_rows, o0, o1)

        @pl.when(j == UNITS - 1)
        def _():
            ob_bh[b] = ob[...] / jnp.sum(lb[...], axis=-1, keepdims=True)

    def out_part(p, j):
        lhs, w = ((ctxa, woa_buf), (ob_hb, wob_buf))[p]
        a = jnp.concatenate([lhs[s * 8 + j] for s in range(4)], axis=1).astype(BF16)
        wait_part(parts_w2, p, j)
        wblk = w[:, unit_rows("n512", j), :].reshape(512, 512)
        return outacc[p] + _dot(a, wblk, NN)

    def step_w2(j):
        @pl.when(j == 0)
        def _():
            ob_hb[...] = jnp.swapaxes(ob_bh[...], 0, 1)
            outacc[...] = jnp.zeros(outacc.shape, F32)

        outacc[0] = out_part(0, j)
        outacc[1] = out_part(1, j)

    xa_cp = pltpu.make_async_copy(xa_hbm, xa_buf, sems.at[2, 4])
    xb_cp = pltpu.make_async_copy(xb_hbm, xb_buf, sems.at[2, 5])
    xa_cp.start()
    xb_cp.start()
    for u in range(LOOKAHEAD):
        start_pair(parts_w0, u)
    xa_cp.wait()
    xb_cp.wait()
    zeros4 = jnp.zeros((4, 512), F32)
    x8_ref[0] = jnp.concatenate([xa_buf[...].astype(F32), zeros4], axis=0)
    x8_ref[1] = jnp.concatenate([xb_buf[...].astype(F32), zeros4], axis=0)

    def body(u, carry):
        issue(u + LOOKAHEAD)
        dispatch(u, step_w0, step_w1, step_c, step_k, step_v, step_w2)
        return carry

    lax.fori_loop(0, N_UNITS - 1, body, 0)

    j = UNITS - 1
    out_ref[:, 0:512] = out_part(0, j)[0:4].astype(out_ref.dtype)
    acc = outacc[1]
    for s in range(4):
        a = ob_hb[s * 8 + j].astype(BF16)
        view = wob_buf.at[s, pl.ds(j * 128, 128), :]
        pltpu.make_async_copy(view, view, sems.at[2, s]).wait()
        acc = acc + _dot(a, view[...], NN)
    out_ref[:, 512:1024] = acc[0:4].astype(out_ref.dtype)


@jax.jit
def pallas_concat_heads__compressed_kv_cla__gqa_block_cached__decode_kernel(
    A_x: jax.Array,
    A_c_kv: jax.Array,
    A_w_q: jax.Array,
    A_w_uk: jax.Array,
    A_w_uv: jax.Array,
    A_w_o: jax.Array,
    B_x: jax.Array,
    B_k_cache: jax.Array,
    B_v_cache: jax.Array,
    B_wq: jax.Array,
    B_wo: jax.Array,
):
    args = (
        A_x.reshape(4, 512),
        A_c_kv.reshape(16, 1024, 512),
        A_w_q.reshape(4, 4096, 128),
        A_w_uk.reshape(4, 4096, 128),
        A_w_uv.reshape(4, 4096, 128),
        A_w_o.reshape(4, 1024, 512),
        B_x.reshape(4, 512),
        B_k_cache.reshape(32, 4096, 128),
        B_v_cache.reshape(32, 4096, 128),
        B_wq.reshape(4, 128, 4096),
        B_wo.reshape(4, 1024, 512),
    )
    vm = pltpu.VMEM
    scratch = [
        vm((4, 512), BF16), vm((4, 512), BF16),
        vm((4, 4096, 128), BF16), vm((4, 4096, 128), BF16), vm((4, 4096, 128), BF16),
        vm((32, 512, 128), BF16), vm((32, 512, 128), BF16), vm((32, 512, 128), BF16),
        vm((4, 128, 4096), BF16),
        vm((4, 1024, 512), BF16), vm((4, 1024, 512), BF16),
        vm((8, 4096, 128), BF16), vm((8, 4096, 128), BF16),
        vm((16, 1024, 512), BF16),
        vm((2, 8, 512), F32),
        vm((32, 8, 512), F32),
        vm((4, 32, 512), BF16),
        vm((32, 8, 128), F32),
        vm((4, 32, 128), F32),
        vm((8, 32, 512), F32),
        vm((32, 128), F32), vm((32, 128), F32), vm((32, 128), F32),
        vm((8, 32, 128), F32), vm((32, 8, 128), F32),
        vm((4, 8, 32, 512), F32),
        vm((4, 32, 128), F32), vm((4, 32, 128), F32), vm((4, 32, 512), F32),
        vm((32, 8, 512), F32), vm((32, 8, 128), F32),
        vm((2, 8, 512), F32),
        pltpu.SemaphoreType.DMA((3, UNITS)),
    ]
    out = pl.pallas_call(
        _kernel,
        out_shape=jax.ShapeDtypeStruct((4, 1024), A_x.dtype),
        in_specs=[pl.BlockSpec(memory_space=pl.ANY)] * 11,
        out_specs=pl.BlockSpec(memory_space=pltpu.VMEM),
        scratch_shapes=scratch,
        compiler_params=pltpu.CompilerParams(
            vmem_limit_bytes=100 * 1024 * 1024,
            disable_bounds_checks=True,
            disable_semaphore_checks=True,
        ),
    )(*args)
    return out.reshape(4, 1, 1024)
```

```python
import jax
import jax.numpy as jnp
from jax import lax
import jax.experimental.pallas as pl
import jax.experimental.pallas.tpu as pltpu

F32 = jnp.float32
BF16 = jnp.bfloat16
NT = (((1,), (1,)), ((), ()))
NN = (((1,), (0,)), ((), ()))

UNITS = 8
G_W0, G_W1, G_M0, G_W2 = 0, 1, 2, 10
N_UNITS = (G_W2 + 1) * UNITS
LOOKAHEAD = 5


def _dot(a, b, dims):
    return lax.dot_general(a, b, dims, preferred_element_type=F32)


def _fold_lanes(x, op):
    r = x[:, 0:128]
    for t in range(1, x.shape[1] // 128):
        r = op(r, x[:, t * 128:(t + 1) * 128])
    return r


def _kernel(xa_hbm, ckv_hbm, wqa_hbm, wuk_hbm, wuv_hbm, woa_hbm,
            xb_hbm, k_hbm, v_hbm, wqb_hbm, wob_hbm,
            out_ref,
            xa_buf, xb_buf, wqa_raw, wuk_raw, wuv_raw, wqa_t, wuk_t, wuv_t,
            wqb_buf, wo_buf, kvbuf, cbuf,
            x8_ref, ql_hb, qlat, qb, mb, lb, ob,
            ma, la, acca, cl_bh, cl_hb, olhs, outacc,
            sems):
    scale = 128.0 ** -0.5

    def piece(kind, j, i):
        if kind == "n128":
            return pl.ds(pl.multiple_of(j * 512 + i * 128, 128), 128), slice(None)
        if kind == "n512":
            return pl.ds(pl.multiple_of(j * 128 + i * 32, 32), 32), slice(None)
        return (pl.ds(pl.multiple_of(j * 16 + (i // 2) * 8, 8), 8),
                pl.ds((i % 2) * 2048, 2048))

    def unit_rows(kind, j):
        n = {"n128": 512, "n512": 128, "wide": 16}[kind]
        return pl.ds(pl.multiple_of(j * n, n), n)

    def start_piece(src, s_src, dst, s_dst, kind, j, i, sem, prio):
        rows, cols = piece(kind, j, i)
        pltpu.make_async_copy(src.at[s_src, rows, cols], dst.at[s_dst, rows, cols],
                              sem).start(priority=prio)

    def wait_rows(dst, kind, j, sem):
        view = dst.at[:, unit_rows(kind, j), :]
        pltpu.make_async_copy(view, view, sem).wait()

    parts_w0 = ((wqa_hbm, wqa_raw, "n128"), (wuk_hbm, wuk_raw, "n128"))
    parts_w1 = ((wuv_hbm, wuv_raw, "n128"), (wqb_hbm, wqb_buf, "wide"))

    def start_pair(parts, j, prio=None):
        for i in range(4):
            for p, (src, dst, kind) in enumerate(parts):
                for s in range(4):
                    start_piece(src, s, dst, s, kind, j, i, sems.at[p, j],
                                s % 2 if prio is None else prio)

    def wait_pair(parts, j):
        for p, (_, dst, kind) in enumerate(parts):
            wait_rows(dst, kind, j, sems.at[p, j])

    def start_main(h, j):
        for i in range(4):
            for t in range(2):
                start_piece(ckv_hbm, h + 8 * t, cbuf, t, "n512", j, i, sems.at[1, j], t)
            for n, src in enumerate((k_hbm, v_hbm)):
                for b in range(4):
                    start_piece(src, h + 8 * b, kvbuf, 4 * n + b, "n128", j, i,
                                sems.at[0, j], b % 2)

    def start_wo_piece(n, j, i, sem):
        src = woa_hbm if n < 4 else wob_hbm
        start_piece(src, n % 4, wo_buf.at[n // 2], n % 2, "n512", j, i, sem, n % 2)

    def start_wo(j):
        for i in range(4):
            for n in range(8):
                start_wo_piece(n, j, i, sems.at[n % 2, j])

    def start_last_unit():
        j = UNITS - 1
        for t in range(16):
            start_wo_piece(2 * (t % 4), j, t // 4, sems.at[0, j])
            start_wo_piece(2 * (t // 4) + 1, j, t % 4, sems.at[2, t // 4])

    def dispatch(u, w0, w1, main, w2):
        g = u // UNITS
        j = u % UNITS
        pl.when(g == G_W0)(lambda: w0(j))
        pl.when(g == G_W1)(lambda: w1(j))
        pl.when(jnp.logical_and(g >= G_M0, g < G_W2))(lambda: main(g - G_M0, j))
        pl.when(jnp.logical_and(g == G_W2, j < UNITS - 1))(lambda: w2(j))

    def issue(u):
        dispatch(u, lambda j: start_pair(parts_w0, j), lambda j: start_pair(parts_w1, j),
                 start_main, start_wo)
        pl.when(u == N_UNITS - 1)(start_last_unit)

    def head_major(raw, dst, j):
        for s in range(4):
            blk = raw[s, unit_rows("n128", j), :].reshape(16, 32, 128)
            d0 = pl.multiple_of(s * 128 + j * 16, 16)
            dst[:, pl.ds(d0, 16), :] = jnp.swapaxes(blk, 0, 1)

    def step_w0(j):
        wait_pair(parts_w0, j)
        head_major(wqa_raw, wqa_t, j)
        head_major(wuk_raw, wuk_t, j)

    def step_w1(j):
        wait_pair(parts_w1, j)
        head_major(wuv_raw, wuv_t, j)
        xa8 = x8_ref[0].astype(BF16)
        for t in range(4):
            h = j * 4 + t
            q = _dot(xa8, wqa_t[h], NN).astype(BF16)
            ql_hb[h] = _dot(q, wuk_t[h], NT) * scale

    row_b = lax.broadcasted_iota(jnp.int32, (16, 1), 0) % 4

    def pick_batch(xs):
        lo = jnp.where(row_b == 0, xs[0], xs[1])
        hi = jnp.where(row_b == 2, xs[2], xs[3])
        return jnp.where(row_b < 2, lo, hi)

    def online_softmax(s, m_old, l_old):
        m_new = jnp.maximum(m_old, jnp.max(s, axis=-1, keepdims=True))
        alpha = jnp.exp(m_old - m_new)
        p = jnp.exp(s - m_new)
        return p, m_new, alpha, alpha * l_old + _fold_lanes(p, jnp.add)

    def step_main(h, j):
        @pl.when(j == 0)
        def _():
            @pl.when(h == 0)
            def _():
                qlat[...] = jnp.swapaxes(ql_hb[...], 0, 1)[0:4].astype(BF16)
                cl_bh[...] = jnp.zeros(cl_bh.shape, F32)
                olhs[...] = jnp.zeros(olhs.shape, F32)

            @pl.when(h % 4 == 0)
            def _():
                ma[...] = jnp.full(ma.shape, -jnp.inf, F32)
                la[...] = jnp.zeros(la.shape, F32)
                acca[...] = jnp.zeros(acca.shape, F32)

            cols = pl.ds(pl.multiple_of(h * 512, 512), 512)
            qc = _dot(x8_ref[1].astype(BF16), wqb_buf[:, :, cols].reshape(512, 512), NN)
            qb[...] = jnp.concatenate(
                [qc[0:4, r * 128:(r + 1) * 128] for r in range(4)], axis=0).astype(BF16)
            mb[...] = jnp.full(mb.shape, -jnp.inf, F32)
            lb[...] = jnp.zeros(lb.shape, F32)
            ob[...] = jnp.zeros(ob.shape, F32)

        wait_rows(kvbuf, "n128", j, sems.at[0, j])
        wait_rows(cbuf, "n512", j, sems.at[1, j])

        rows = unit_rows("n128", j)
        crows = unit_rows("n512", j)
        sa = [_dot(qlat[h // 4 + 2 * t], cbuf[t, crows, :], NT) for t in range(2)]
        q16 = qb[...]
        sb = pick_batch([_dot(q16, kvbuf[b, rows, :], NT) for b in range(4)]) * scale

        for t in range(2):
            p, m_new, alpha, l_new = online_softmax(sa[t], ma[t], la[t])
            ma[t] = m_new
            la[t] = l_new
            acca[t] = alpha * acca[t] + _dot(p.astype(BF16), cbuf[t, crows, :], NN)

        p, m_new, alpha, l_new = online_softmax(sb, mb[...], lb[...])
        p = p.astype(BF16)
        o = pick_batch([_dot(p, kvbuf[4 + b, rows, :], NN) for b in range(4)])
        mb[...] = m_new
        lb[...] = l_new
        ob[...] = alpha * ob[...] + o

        @pl.when(j == UNITS - 1)
        def _():
            o = ob[...] / jnp.sum(lb[...], axis=-1, keepdims=True)
            for r in range(4):
                olhs[32 + 4 * h + r, 0:4, :] = o[4 * r:4 * r + 4]

            @pl.when(h % 4 == 3)
            def _():
                for t in range(2):
                    cl_bh[h // 4 + 2 * t] = acca[t] / jnp.sum(la[t], axis=-1, keepdims=True)

    def out_part(p, j):
        rows = unit_rows("n512", j)
        lhs = [jnp.concatenate([olhs[(4 * a + p) * 8 + j], olhs[(4 * a + p + 2) * 8 + j]],
                               axis=1).astype(BF16) for a in range(2)]
        view = wo_buf.at[:, p, rows, :]
        pltpu.make_async_copy(view, view, sems.at[p, j]).wait()
        for a in range(2):
            wblk = wo_buf[2 * a:2 * a + 2, p, rows, :].reshape(256, 512)
            outacc[a] += _dot(lhs[a], wblk, NN)

    def step_w2(j):
        @pl.when(j == 0)
        def _():
            cl_hb[...] = jnp.swapaxes(cl_bh[...], 0, 1)
            outacc[...] = jnp.zeros(outacc.shape, F32)

        @pl.when(j < 4)
        def _():
            for s in range(4):
                for t in range(2):
                    h = s * 8 + 2 * j + t
                    olhs[h] = _dot(cl_hb[h].astype(BF16), wuv_t[h], NN)

        pl.when(j == 0)(lambda: out_part(0, 0))
        out_part(0, j + 1)
        out_part(1, j)

    xa_cp = pltpu.make_async_copy(xa_hbm, xa_buf, sems.at[2, 4])
    xb_cp = pltpu.make_async_copy(xb_hbm, xb_buf, sems.at[2, 5])
    xa_cp.start()
    xb_cp.start()
    for u in range(LOOKAHEAD):
        start_pair(parts_w0, u, 1 if u == 0 else None)
    xa_cp.wait()
    xb_cp.wait()
    zeros4 = jnp.zeros((4, 512), F32)
    x8_ref[0] = jnp.concatenate([xa_buf[...].astype(F32), zeros4], axis=0)
    x8_ref[1] = jnp.concatenate([xb_buf[...].astype(F32), zeros4], axis=0)

    def body(u, carry):
        issue(u + LOOKAHEAD)
        dispatch(u, step_w0, step_w1, step_main, step_w2)
        return carry

    lax.fori_loop(0, N_UNITS - 1, body, 0)

    j = UNITS - 1
    for a in range(2):
        acc = outacc[a]
        for t in (2 * a, 2 * a + 1):
            lhs = olhs[(2 * t + 1) * 8 + j].astype(BF16)
            view = wo_buf.at[t, 1, pl.ds(j * 128, 128), :]
            pltpu.make_async_copy(view, view, sems.at[2, t]).wait()
            acc = acc + _dot(lhs, view[...], NN)
        out_ref[:, a * 512:(a + 1) * 512] = acc[0:4].astype(out_ref.dtype)


@jax.jit
def pallas_concat_heads__compressed_kv_cla__gqa_block_cached__decode_kernel(
    A_x: jax.Array,
    A_c_kv: jax.Array,
    A_w_q: jax.Array,
    A_w_uk: jax.Array,
    A_w_uv: jax.Array,
    A_w_o: jax.Array,
    B_x: jax.Array,
    B_k_cache: jax.Array,
    B_v_cache: jax.Array,
    B_wq: jax.Array,
    B_wo: jax.Array,
):
    args = (
        A_x.reshape(4, 512),
        A_c_kv.reshape(16, 1024, 512),
        A_w_q.reshape(4, 4096, 128),
        A_w_uk.reshape(4, 4096, 128),
        A_w_uv.reshape(4, 4096, 128),
        A_w_o.reshape(4, 1024, 512),
        B_x.reshape(4, 512),
        B_k_cache.reshape(32, 4096, 128),
        B_v_cache.reshape(32, 4096, 128),
        B_wq.reshape(4, 128, 4096),
        B_wo.reshape(4, 1024, 512),
    )
    vm = pltpu.VMEM
    scratch = [
        vm((4, 512), BF16), vm((4, 512), BF16),
        vm((4, 4096, 128), BF16), vm((4, 4096, 128), BF16), vm((4, 4096, 128), BF16),
        vm((32, 512, 128), BF16), vm((32, 512, 128), BF16), vm((32, 512, 128), BF16),
        vm((4, 128, 4096), BF16),
        vm((4, 2, 1024, 512), BF16),
        vm((8, 4096, 128), BF16),
        vm((2, 1024, 512), BF16),
        vm((2, 8, 512), F32),
        vm((32, 8, 512), F32),
        vm((4, 32, 512), BF16),
        vm((16, 128), BF16),
        vm((16, 1), F32), vm((16, 128), F32), vm((16, 128), F32),
        vm((2, 32, 1), F32), vm((2, 32, 128), F32), vm((2, 32, 512), F32),
        vm((8, 32, 512), F32), vm((32, 8, 512), F32),
        vm((64, 8, 128), F32),
        vm((2, 8, 512), F32),
        pltpu.SemaphoreType.DMA((3, UNITS)),
    ]
    out = pl.pallas_call(
        _kernel,
        out_shape=jax.ShapeDtypeStruct((4, 1024), A_x.dtype),
        in_specs=[pl.BlockSpec(memory_space=pl.ANY)] * 11,
        out_specs=pl.BlockSpec(memory_space=pltpu.VMEM),
        scratch_shapes=scratch,
        compiler_params=pltpu.CompilerParams(
            vmem_limit_bytes=100 * 1024 * 1024,
            disable_bounds_checks=True,
            disable_semaphore_checks=True,
        ),
    )(*args)
    return out.reshape(4, 1, 1024)
```

```python
import jax
import jax.numpy as jnp
from jax import lax
import jax.experimental.pallas as pl
import jax.experimental.pallas.tpu as pltpu

F32 = jnp.float32
BF16 = jnp.bfloat16
NT = (((1,), (1,)), ((), ()))
NN = (((1,), (0,)), ((), ()))

UNITS = 8
G_W0, G_W1, G_M0, G_W2 = 0, 1, 2, 10
N_UNITS = (G_W2 + 1) * UNITS
LOOKAHEAD = 5
KV_SHIFT = 8


def _dot(a, b, dims):
    return lax.dot_general(a, b, dims, preferred_element_type=F32)


def _fold_lanes(x, op):
    r = x[:, 0:128]
    for t in range(1, x.shape[1] // 128):
        r = op(r, x[:, t * 128:(t + 1) * 128])
    return r


def _kernel(xa_hbm, ckv_hbm, wqa_hbm, wuk_hbm, wuv_hbm, woa_hbm,
            xb_hbm, k_hbm, v_hbm, wqb_hbm, wob_hbm,
            out_ref,
            xa_buf, xb_buf, wqa_raw, wuk_raw, wuv_raw, wqa_t, wuk_t, wuv_t,
            wqb_buf, wo_buf, kvbuf, cbuf,
            x8_ref, ql_hb, qlat, qb, mb, lb, ob,
            ma, la, acca, cl_bh, cl_hb, olhs, outacc,
            sems):
    scale = 128.0 ** -0.5

    def piece(kind, j, i):
        if kind == "n128":
            return pl.ds(pl.multiple_of(j * 512 + i * 128, 128), 128), slice(None)
        if kind == "n512":
            return pl.ds(pl.multiple_of(j * 128 + i * 32, 32), 32), slice(None)
        return (pl.ds(pl.multiple_of(j * 16 + (i // 2) * 8, 8), 8),
                pl.ds((i % 2) * 2048, 2048))

    def unit_rows(kind, j):
        n = {"n128": 512, "n512": 128, "wide": 16}[kind]
        return pl.ds(pl.multiple_of(j * n, n), n)

    def start_piece(src, s_src, dst, s_dst, kind, j, i, sem, prio):
        rows, cols = piece(kind, j, i)
        pltpu.make_async_copy(src.at[s_src, rows, cols], dst.at[s_dst, rows, cols],
                              sem).start(priority=prio)

    def wait_rows(dst, kind, j, sem):
        view = dst.at[:, unit_rows(kind, j), :]
        pltpu.make_async_copy(view, view, sem).wait()

    parts_w0 = ((wqa_hbm, wqa_raw, "n128"), (wuk_hbm, wuk_raw, "n128"))
    parts_w1 = ((wuv_hbm, wuv_raw, "n128"), (wqb_hbm, wqb_buf, "wide"))

    def start_pair(parts, j, prio=None):
        for i in range(4):
            for p, (src, dst, kind) in enumerate(parts):
                for s in range(4):
                    start_piece(src, s, dst, s, kind, j, i, sems.at[p, j],
                                s % 2 if prio is None else prio)

    def wait_pair(parts, j):
        for p, (_, dst, kind) in enumerate(parts):
            wait_rows(dst, kind, j, sems.at[p, j])

    def start_kv_rows(h, r0, n, sem):
        rows = pl.ds(pl.multiple_of(r0, 8), n)
        for t, src in enumerate((k_hbm, v_hbm)):
            for b in range(4):
                pltpu.make_async_copy(src.at[h + 8 * b, rows, :], kvbuf.at[4 * t + b, rows, :],
                                      sem).start(priority=b % 2)

    def wait_kv_rows(r0, n, sem):
        view = kvbuf.at[:, pl.ds(pl.multiple_of(r0, 8), n), :]
        pltpu.make_async_copy(view, view, sem).wait()

    c_cols = (pl.ds(384, 128), pl.ds(0, 384))

    def start_c(h, regions, slot):
        for t in range(2):
            for k, (r0, n) in enumerate(regions):
                rows = pl.ds(pl.multiple_of(r0, 8), n)
                pltpu.make_async_copy(ckv_hbm.at[h + 8 * t, rows, c_cols[k]],
                                      cbuf.at[t, rows, c_cols[k]],
                                      sems.at[1 + k, slot]).start(priority=t)

    def wait_c(regions, slot):
        for k, (r0, n) in enumerate(regions):
            view = cbuf.at[:, pl.ds(pl.multiple_of(r0, 8), n), c_cols[k]]
            pltpu.make_async_copy(view, view, sems.at[1 + k, slot]).wait()

    last = UNITS - 1
    head = UNITS

    def start_main(h, j):
        @pl.when(j == 0)
        def _():
            start_c(h, ((0, 24), (0, 32)), head)
            start_kv_rows(h, 0, KV_SHIFT, sems.at[0, head])

        def full_round(i):
            r = j * 128 + i * 32 + 32
            start_c(h, ((r - 8, 32), (r, 32)), j)
            start_kv_rows(h, j * 512 + i * 128 + KV_SHIFT, 128, sems.at[0, j])

        for i in range(3):
            full_round(i)
        pl.when(j < last)(lambda: full_round(3))

        @pl.when(j == last)
        def _():
            start_c(h, ((1016, 8),), last)
            start_kv_rows(h, 3968 + KV_SHIFT, 128 - KV_SHIFT, sems.at[0, last])

    def wait_main(j):
        @pl.when(j == 0)
        def _():
            wait_c(((0, 24), (0, 32)), head)
            wait_kv_rows(0, KV_SHIFT, sems.at[0, head])

        @pl.when(j < last)
        def _():
            wait_kv_rows(j * 512 + KV_SHIFT, 512, sems.at[0, j])
            wait_c(((j * 128 + 24, 128), (j * 128 + 32, 128)), j)

        @pl.when(j == last)
        def _():
            wait_kv_rows(3584 + KV_SHIFT, 512 - KV_SHIFT, sems.at[0, last])
            wait_c(((920, 104), (928, 96)), last)

    def start_wo_piece(n, j, i, sem):
        src = woa_hbm if n < 4 else wob_hbm
        start_piece(src, n % 4, wo_buf.at[n // 2], n % 2, "n512", j, i, sem, n % 2)

    def start_wo(j):
        for i in range(4):
            for n in range(8):
                start_wo_piece(n, j, i, sems.at[n % 2, j])

    def start_last_unit():
        j = UNITS - 1
        for t in range(16):
            start_wo_piece(2 * (t % 4), j, t // 4, sems.at[0, j])
            start_wo_piece(2 * (t // 4) + 1, j, t % 4, sems.at[3, t // 4])

    def dispatch(u, w0, w1, main, w2):
        g = u // UNITS
        j = u % UNITS
        pl.when(g == G_W0)(lambda: w0(j))
        pl.when(g == G_W1)(lambda: w1(j))
        pl.when(jnp.logical_and(g >= G_M0, g < G_W2))(lambda: main(g - G_M0, j))
        pl.when(jnp.logical_and(g == G_W2, j < UNITS - 1))(lambda: w2(j))

    def issue(u):
        dispatch(u, lambda j: start_pair(parts_w0, j), lambda j: start_pair(parts_w1, j),
                 start_main, start_wo)
        pl.when(u == N_UNITS - 1)(start_last_unit)

    def head_major(raw, dst, j):
        for s in range(4):
            blk = raw[s, unit_rows("n128", j), :].reshape(16, 32, 128)
            d0 = pl.multiple_of(s * 128 + j * 16, 16)
            dst[:, pl.ds(d0, 16), :] = jnp.swapaxes(blk, 0, 1)

    def step_w0(j):
        wait_pair(parts_w0, j)
        head_major(wqa_raw, wqa_t, j)
        head_major(wuk_raw, wuk_t, j)

    def step_w1(j):
        wait_pair(parts_w1, j)
        head_major(wuv_raw, wuv_t, j)
        xa8 = x8_ref[0].astype(BF16)
        for t in range(4):
            h = j * 4 + t
            q = _dot(xa8, wqa_t[h], NN).astype(BF16)
            ql_hb[h] = _dot(q, wuk_t[h], NT) * scale

    row_b = lax.broadcasted_iota(jnp.int32, (16, 1), 0) % 4

    def pick_batch(xs):
        lo = jnp.where(row_b == 0, xs[0], xs[1])
        hi = jnp.where(row_b == 2, xs[2], xs[3])
        return jnp.where(row_b < 2, lo, hi)

    def online_softmax(s, m_old, l_old):
        m_new = jnp.maximum(m_old, jnp.max(s, axis=-1, keepdims=True))
        alpha = jnp.exp(m_old - m_new)
        p = jnp.exp(s - m_new)
        return p, m_new, alpha, alpha * l_old + _fold_lanes(p, jnp.add)

    def step_main(h, j):
        @pl.when(j == 0)
        def _():
            @pl.when(h == 0)
            def _():
                qlat[...] = jnp.swapaxes(ql_hb[...], 0, 1)[0:4].astype(BF16)
                cl_bh[...] = jnp.zeros(cl_bh.shape, F32)
                olhs[...] = jnp.zeros(olhs.shape, F32)

            @pl.when(h % 4 == 0)
            def _():
                ma[...] = jnp.full(ma.shape, -jnp.inf, F32)
                la[...] = jnp.zeros(la.shape, F32)
                acca[...] = jnp.zeros(acca.shape, F32)

            cols = pl.ds(pl.multiple_of(h * 512, 512), 512)
            qc = _dot(x8_ref[1].astype(BF16), wqb_buf[:, :, cols].reshape(512, 512), NN)
            qb[...] = jnp.concatenate(
                [qc[0:4, r * 128:(r + 1) * 128] for r in range(4)], axis=0).astype(BF16)
            mb[...] = jnp.full(mb.shape, -jnp.inf, F32)
            lb[...] = jnp.zeros(lb.shape, F32)
            ob[...] = jnp.zeros(ob.shape, F32)

        wait_main(j)

        rows = unit_rows("n128", j)
        crows = unit_rows("n512", j)
        sa = [_dot(qlat[h // 4 + 2 * t], cbuf[t, crows, :], NT) for t in range(2)]
        q16 = qb[...]
        sb = pick_batch([_dot(q16, kvbuf[b, rows, :], NT) for b in range(4)]) * scale

        for t in range(2):
            p, m_new, alpha, l_new = online_softmax(sa[t], ma[t], la[t])
            ma[t] = m_new
            la[t] = l_new
            acca[t] = alpha * acca[t] + _dot(p.astype(BF16), cbuf[t, crows, :], NN)

        p, m_new, alpha, l_new = online_softmax(sb, mb[...], lb[...])
        p = p.astype(BF16)
        o = pick_batch([_dot(p, kvbuf[4 + b, rows, :], NN) for b in range(4)])
        mb[...] = m_new
        lb[...] = l_new
        ob[...] = alpha * ob[...] + o

        @pl.when(j == UNITS - 1)
        def _():
            o = ob[...] / jnp.sum(lb[...], axis=-1, keepdims=True)
            for r in range(4):
                olhs[32 + 4 * h + r, 0:4, :] = o[4 * r:4 * r + 4]

            @pl.when(h % 4 == 3)
            def _():
                for t in range(2):
                    cl_bh[h // 4 + 2 * t] = acca[t] / jnp.sum(la[t], axis=-1, keepdims=True)

    def out_part(p, j):
        rows = unit_rows("n512", j)
        lhs = [jnp.concatenate([olhs[(4 * a + p) * 8 + j], olhs[(4 * a + p + 2) * 8 + j]],
                               axis=1).astype(BF16) for a in range(2)]
        view = wo_buf.at[:, p, rows, :]
        pltpu.make_async_copy(view, view, sems.at[p, j]).wait()
        for a in range(2):
            wblk = wo_buf[2 * a:2 * a + 2, p, rows, :].reshape(256, 512)
            outacc[a] += _dot(lhs[a], wblk, NN)

    def step_w2(j):
        @pl.when(j == 0)
        def _():
            cl_hb[...] = jnp.swapaxes(cl_bh[...], 0, 1)
            outacc[...] = jnp.zeros(outacc.shape, F32)

        @pl.when(j < 4)
        def _():
            for s in range(4):
                for t in range(2):
                    h = s * 8 + 2 * j + t
                    olhs[h] = _dot(cl_hb[h].astype(BF16), wuv_t[h], NN)

        pl.when(j == 0)(lambda: out_part(0, 0))
        out_part(0, j + 1)
        out_part(1, j)

    xa_cp = pltpu.make_async_copy(xa_hbm, xa_buf, sems.at[3, 4])
    xb_cp = pltpu.make_async_copy(xb_hbm, xb_buf, sems.at[3, 5])
    xa_cp.start()
    xb_cp.start()
    for u in range(LOOKAHEAD):
        start_pair(parts_w0, u, 1 if u == 0 else None)
    xa_cp.wait()
    xb_cp.wait()
    zeros4 = jnp.zeros((4, 512), F32)
    x8_ref[0] = jnp.concatenate([xa_buf[...].astype(F32), zeros4], axis=0)
    x8_ref[1] = jnp.concatenate([xb_buf[...].astype(F32), zeros4], axis=0)

    def body(u, carry):
        issue(u + LOOKAHEAD)
        dispatch(u, step_w0, step_w1, step_main, step_w2)
        return carry

    lax.fori_loop(0, N_UNITS - 1, body, 0)

    j = UNITS - 1
    for a in range(2):
        acc = outacc[a]
        for t in (2 * a, 2 * a + 1):
            lhs = olhs[(2 * t + 1) * 8 + j].astype(BF16)
            view = wo_buf.at[t, 1, pl.ds(j * 128, 128), :]
            pltpu.make_async_copy(view, view, sems.at[3, t]).wait()
            acc = acc + _dot(lhs, view[...], NN)
        out_ref[:, a * 512:(a + 1) * 512] = acc[0:4].astype(out_ref.dtype)


@jax.jit
def pallas_concat_heads__compressed_kv_cla__gqa_block_cached__decode_kernel(
    A_x: jax.Array,
    A_c_kv: jax.Array,
    A_w_q: jax.Array,
    A_w_uk: jax.Array,
    A_w_uv: jax.Array,
    A_w_o: jax.Array,
    B_x: jax.Array,
    B_k_cache: jax.Array,
    B_v_cache: jax.Array,
    B_wq: jax.Array,
    B_wo: jax.Array,
):
    args = (
        A_x.reshape(4, 512),
        A_c_kv.reshape(16, 1024, 512),
        A_w_q.reshape(4, 4096, 128),
        A_w_uk.reshape(4, 4096, 128),
        A_w_uv.reshape(4, 4096, 128),
        A_w_o.reshape(4, 1024, 512),
        B_x.reshape(4, 512),
        B_k_cache.reshape(32, 4096, 128),
        B_v_cache.reshape(32, 4096, 128),
        B_wq.reshape(4, 128, 4096),
        B_wo.reshape(4, 1024, 512),
    )
    vm = pltpu.VMEM
    scratch = [
        vm((4, 512), BF16), vm((4, 512), BF16),
        vm((4, 4096, 128), BF16), vm((4, 4096, 128), BF16), vm((4, 4096, 128), BF16),
        vm((32, 512, 128), BF16), vm((32, 512, 128), BF16), vm((32, 512, 128), BF16),
        vm((4, 128, 4096), BF16),
        vm((4, 2, 1024, 512), BF16),
        vm((8, 4096, 128), BF16),
        vm((2, 1024, 512), BF16),
        vm((2, 8, 512), F32),
        vm((32, 8, 512), F32),
        vm((4, 32, 512), BF16),
        vm((16, 128), BF16),
        vm((16, 1), F32), vm((16, 128), F32), vm((16, 128), F32),
        vm((2, 32, 1), F32), vm((2, 32, 128), F32), vm((2, 32, 512), F32),
        vm((8, 32, 512), F32), vm((32, 8, 512), F32),
        vm((64, 8, 128), F32),
        vm((2, 8, 512), F32),
        pltpu.SemaphoreType.DMA((4, UNITS + 1)),
    ]
    out = pl.pallas_call(
        _kernel,
        out_shape=jax.ShapeDtypeStruct((4, 1024), A_x.dtype),
        in_specs=[pl.BlockSpec(memory_space=pl.ANY)] * 11,
        out_specs=pl.BlockSpec(memory_space=pltpu.VMEM),
        scratch_shapes=scratch,
        compiler_params=pltpu.CompilerParams(
            vmem_limit_bytes=100 * 1024 * 1024,
            disable_bounds_checks=True,
            disable_semaphore_checks=True,
        ),
    )(*args)
    return out.reshape(4, 1, 1024)
```

```python
import jax
import jax.numpy as jnp
from jax import lax
import jax.experimental.pallas as pl
import jax.experimental.pallas.tpu as pltpu

F32 = jnp.float32
BF16 = jnp.bfloat16
NT = (((1,), (1,)), ((), ()))
NN = (((1,), (0,)), ((), ()))

UNITS = 8
G_W0, G_W1, G_M0, G_W2 = 0, 1, 2, 10
N_UNITS = (G_W2 + 1) * UNITS
LOOKAHEAD = 5
KV_SHIFT = 8
W_SHIFT = 8


def _dot(a, b, dims):
    return lax.dot_general(a, b, dims, preferred_element_type=F32)


def _fold_lanes(x, op):
    r = x[:, 0:128]
    for t in range(1, x.shape[1] // 128):
        r = op(r, x[:, t * 128:(t + 1) * 128])
    return r


def _kernel(xa_hbm, ckv_hbm, wqa_hbm, wuk_hbm, wuv_hbm, woa_hbm,
            xb_hbm, k_hbm, v_hbm, wqb_hbm, wob_hbm,
            out_ref,
            xa_buf, xb_buf, wqa_raw, wuk_raw, wuv_raw, wqa_t, wuk_t, wuv_t,
            wqb_buf, wo_buf, kvbuf, cbuf,
            x8_ref, ql_hb, qlat, qb, mb, lb, ob,
            ma, la, acca, cl_bh, cl_hb, olhs, outacc,
            sems):
    scale = 128.0 ** -0.5

    def piece(kind, j, i):
        if kind == "n128":
            return pl.ds(pl.multiple_of(j * 512 + i * 128, 128), 128), slice(None)
        if kind == "n512":
            return pl.ds(pl.multiple_of(j * 128 + i * 32, 32), 32), slice(None)
        return (pl.ds(pl.multiple_of(j * 16 + (i // 2) * 8, 8), 8),
                pl.ds((i % 2) * 2048, 2048))

    def unit_rows(kind, j):
        n = {"n128": 512, "n512": 128, "wide": 16}[kind]
        return pl.ds(pl.multiple_of(j * n, n), n)

    def start_piece(src, s_src, dst, s_dst, kind, j, i, sem, prio):
        rows, cols = piece(kind, j, i)
        pltpu.make_async_copy(src.at[s_src, rows, cols], dst.at[s_dst, rows, cols],
                              sem).start(priority=prio)

    def wait_rows(dst, kind, j, sem):
        view = dst.at[:, unit_rows(kind, j), :]
        pltpu.make_async_copy(view, view, sem).wait()

    parts_w0 = ((wqa_hbm, wqa_raw, "n128"), (wuk_hbm, wuk_raw, "n128"))
    parts_w1 = ((wuv_hbm, wuv_raw, "n128"), (wqb_hbm, wqb_buf, "wide"))

    def start_rolled(src, dst, s, j, i, sem, prio):
        def copy(r_src, r_dst, n):
            pltpu.make_async_copy(src.at[pl.ds(pl.multiple_of(r_src, 8), n), :],
                                  dst.at[s, pl.ds(pl.multiple_of(r_dst, 8), n), :],
                                  sem).start(priority=prio)

        def whole():
            copy(s * 4096 + j * 512 + i * 128 - W_SHIFT, j * 512 + i * 128, 128)

        def wrapped():
            copy(0, W_SHIFT, 128 - W_SHIFT)
            copy(16384 - W_SHIFT, 0, W_SHIFT)

        if s > 0 or i > 0:
            whole()
        elif isinstance(j, int):
            wrapped() if j == 0 else whole()
        else:
            pl.when(j == 0)(wrapped)
            pl.when(j > 0)(whole)

    def start_pair(parts, j, prio=None):
        for i in range(4):
            for p, (src, dst, kind) in enumerate(parts):
                for s in range(4):
                    pr = s % 2 if prio is None else prio
                    if kind == "n128":
                        start_rolled(src, dst, s, j, i, sems.at[p, j], pr)
                    else:
                        start_piece(src, s, dst, s, kind, j, i, sems.at[p, j], pr)

    def wait_pair(parts, j):
        for p, (_, dst, kind) in enumerate(parts):
            wait_rows(dst, kind, j, sems.at[p, j])

    def start_kv_rows(h, r0, n, sem):
        rows = pl.ds(pl.multiple_of(r0, 8), n)
        for t, src in enumerate((k_hbm, v_hbm)):
            for b in range(4):
                pltpu.make_async_copy(src.at[h + 8 * b, rows, :], kvbuf.at[4 * t + b, rows, :],
                                      sem).start(priority=b % 2)

    def wait_kv_rows(r0, n, sem):
        view = kvbuf.at[:, pl.ds(pl.multiple_of(r0, 8), n), :]
        pltpu.make_async_copy(view, view, sem).wait()

    c_cols = (pl.ds(384, 128), pl.ds(0, 384))

    def start_c(h, regions, slot):
        for t in range(2):
            for k, (r0, n) in enumerate(regions):
                rows = pl.ds(pl.multiple_of(r0, 8), n)
                pltpu.make_async_copy(ckv_hbm.at[h + 8 * t, rows, c_cols[k]],
                                      cbuf.at[t, rows, c_cols[k]],
                                      sems.at[1 + k, slot]).start(priority=t)

    def wait_c(regions, slot):
        for k, (r0, n) in enumerate(regions):
            view = cbuf.at[:, pl.ds(pl.multiple_of(r0, 8), n), c_cols[k]]
            pltpu.make_async_copy(view, view, sems.at[1 + k, slot]).wait()

    last = UNITS - 1
    head = UNITS

    def start_main(h, j):
        @pl.when(j == 0)
        def _():
            start_c(h, ((0, 24), (0, 32)), head)
            start_kv_rows(h, 0, KV_SHIFT, sems.at[0, head])

        def full_round(i):
            r = j * 128 + i * 32 + 32
            start_c(h, ((r - 8, 32), (r, 32)), j)
            start_kv_rows(h, j * 512 + i * 128 + KV_SHIFT, 128, sems.at[0, j])

        for i in range(3):
            full_round(i)
        pl.when(j < last)(lambda: full_round(3))

        @pl.when(j == last)
        def _():
            start_c(h, ((1016, 8),), last)
            start_kv_rows(h, 3968 + KV_SHIFT, 128 - KV_SHIFT, sems.at[0, last])

    def wait_main(j):
        @pl.when(j == 0)
        def _():
            wait_c(((0, 24), (0, 32)), head)
            wait_kv_rows(0, KV_SHIFT, sems.at[0, head])

        @pl.when(j < last)
        def _():
            wait_kv_rows(j * 512 + KV_SHIFT, 512, sems.at[0, j])
            wait_c(((j * 128 + 24, 128), (j * 128 + 32, 128)), j)

        @pl.when(j == last)
        def _():
            wait_kv_rows(3584 + KV_SHIFT, 512 - KV_SHIFT, sems.at[0, last])
            wait_c(((920, 104), (928, 96)), last)

    def start_wo_piece(n, j, i, sem):
        src = woa_hbm if n < 4 else wob_hbm
        start_piece(src, n % 4, wo_buf.at[n // 2], n % 2, "n512", j, i, sem, n % 2)

    def start_wo(j):
        for i in range(4):
            for n in range(8):
                start_wo_piece(n, j, i, sems.at[n % 2, j])

    def start_last_unit():
        j = UNITS - 1
        for t in range(16):
            start_wo_piece(2 * (t % 4), j, t // 4, sems.at[0, j])
            start_wo_piece(2 * (t // 4) + 1, j, t % 4, sems.at[3, t // 4])

    def dispatch(u, w0, w1, main, w2):
        g = u // UNITS
        j = u % UNITS
        pl.when(g == G_W0)(lambda: w0(j))
        pl.when(g == G_W1)(lambda: w1(j))
        pl.when(jnp.logical_and(g >= G_M0, g < G_W2))(lambda: main(g - G_M0, j))
        pl.when(jnp.logical_and(g == G_W2, j < UNITS - 1))(lambda: w2(j))

    def issue(u):
        dispatch(u, lambda j: start_pair(parts_w0, j), lambda j: start_pair(parts_w1, j),
                 start_main, start_wo)
        pl.when(u == N_UNITS - 1)(start_last_unit)

    def head_major(raw, dst, j):
        for s in range(4):
            blk = raw[s, unit_rows("n128", j), :].reshape(16, 32, 128)
            d0 = pl.multiple_of(s * 128 + j * 16, 16)
            dst[:, pl.ds(d0, 16), :] = jnp.swapaxes(blk, 0, 1)

    def step_w0(j):
        wait_pair(parts_w0, j)
        head_major(wqa_raw, wqa_t, j)
        head_major(wuk_raw, wuk_t, j)

    def step_w1(j):
        wait_pair(parts_w1, j)
        head_major(wuv_raw, wuv_t, j)
        xa8 = x8_ref[0]
        for s in range(4):
            slot = ((s + 1) % 4) * 8 + j
            x = pltpu.roll(xa8, 1, 1) if s == 3 else xa8
            q = _dot(x.astype(BF16), wqa_t[slot], NN).astype(BF16)
            ql = _dot(q, wuk_t[slot], NT) * scale
            ql_hb[s * 8 + j] = pltpu.roll(ql, 511, 1) if s == 3 else ql

    row_b = lax.broadcasted_iota(jnp.int32, (16, 1), 0) % 4

    def pick_batch(xs):
        lo = jnp.where(row_b == 0, xs[0], xs[1])
        hi = jnp.where(row_b == 2, xs[2], xs[3])
        return jnp.where(row_b < 2, lo, hi)

    def online_softmax(s, m_old, l_old):
        m_new = jnp.maximum(m_old, jnp.max(s, axis=-1, keepdims=True))
        alpha = jnp.exp(m_old - m_new)
        p = jnp.exp(s - m_new)
        return p, m_new, alpha, alpha * l_old + _fold_lanes(p, jnp.add)

    def step_main(h, j):
        @pl.when(j == 0)
        def _():
            @pl.when(h == 0)
            def _():
                qlat[...] = jnp.swapaxes(ql_hb[...], 0, 1)[0:4].astype(BF16)
                cl_bh[...] = jnp.zeros(cl_bh.shape, F32)
                olhs[...] = jnp.zeros(olhs.shape, F32)

            @pl.when(h % 4 == 0)
            def _():
                ma[...] = jnp.full(ma.shape, -jnp.inf, F32)
                la[...] = jnp.zeros(la.shape, F32)
                acca[...] = jnp.zeros(acca.shape, F32)

            cols = pl.ds(pl.multiple_of(h * 512, 512), 512)
            qc = _dot(x8_ref[1].astype(BF16), wqb_buf[:, :, cols].reshape(512, 512), NN)
            qb[...] = jnp.concatenate(
                [qc[0:4, r * 128:(r + 1) * 128] for r in range(4)], axis=0).astype(BF16)
            mb[...] = jnp.full(mb.shape, -jnp.inf, F32)
            lb[...] = jnp.zeros(lb.shape, F32)
            ob[...] = jnp.zeros(ob.shape, F32)

        wait_main(j)

        rows = unit_rows("n128", j)
        crows = unit_rows("n512", j)
        sa = [_dot(qlat[h // 4 + 2 * t], cbuf[t, crows, :], NT) for t in range(2)]
        q16 = qb[...]
        sb = pick_batch([_dot(q16, kvbuf[b, rows, :], NT) for b in range(4)]) * scale

        for t in range(2):
            p, m_new, alpha, l_new = online_softmax(sa[t], ma[t], la[t])
            ma[t] = m_new
            la[t] = l_new
            acca[t] = alpha * acca[t] + _dot(p.astype(BF16), cbuf[t, crows, :], NN)

        p, m_new, alpha, l_new = online_softmax(sb, mb[...], lb[...])
        p = p.astype(BF16)
        o = pick_batch([_dot(p, kvbuf[4 + b, rows, :], NN) for b in range(4)])
        mb[...] = m_new
        lb[...] = l_new
        ob[...] = alpha * ob[...] + o

        @pl.when(j == UNITS - 1)
        def _():
            o = ob[...] / jnp.sum(lb[...], axis=-1, keepdims=True)
            for r in range(4):
                olhs[32 + 4 * h + r, 0:4, :] = o[4 * r:4 * r + 4]

            @pl.when(h % 4 == 3)
            def _():
                for t in range(2):
                    cl_bh[h // 4 + 2 * t] = acca[t] / jnp.sum(la[t], axis=-1, keepdims=True)

    def out_part(p, j):
        rows = unit_rows("n512", j)
        lhs = [jnp.concatenate([olhs[(4 * a + p) * 8 + j], olhs[(4 * a + p + 2) * 8 + j]],
                               axis=1).astype(BF16) for a in range(2)]
        view = wo_buf.at[:, p, rows, :]
        pltpu.make_async_copy(view, view, sems.at[p, j]).wait()
        for a in range(2):
            wblk = wo_buf[2 * a:2 * a + 2, p, rows, :].reshape(256, 512)
            outacc[a] += _dot(lhs[a], wblk, NN)

    def step_w2(j):
        @pl.when(j == 0)
        def _():
            cl_hb[...] = jnp.swapaxes(cl_bh[...], 0, 1)
            outacc[...] = jnp.zeros(outacc.shape, F32)

        @pl.when(j < 4)
        def _():
            for s in range(4):
                for t in range(2):
                    c = 2 * j + t
                    cl = cl_hb[s * 8 + c]
                    cl = pltpu.roll(cl, 1, 1) if s == 3 else cl
                    w = wuv_t[((s + 1) % 4) * 8 + c]
                    olhs[s * 8 + c] = _dot(cl.astype(BF16), w, NN)

        pl.when(j == 0)(lambda: out_part(0, 0))
        out_part(0, j + 1)
        out_part(1, j)

    xa_cp = pltpu.make_async_copy(xa_hbm, xa_buf, sems.at[3, 4])
    xb_cp = pltpu.make_async_copy(xb_hbm, xb_buf, sems.at[3, 5])
    xa_cp.start()
    xb_cp.start()
    for u in range(LOOKAHEAD):
        start_pair(parts_w0, u, 1 if u == 0 else None)
    xa_cp.wait()
    xb_cp.wait()
    zeros4 = jnp.zeros((4, 512), F32)
    x8_ref[0] = jnp.concatenate([xa_buf[...].astype(F32), zeros4], axis=0)
    x8_ref[1] = jnp.concatenate([xb_buf[...].astype(F32), zeros4], axis=0)

    def body(u, carry):
        issue(u + LOOKAHEAD)
        dispatch(u, step_w0, step_w1, step_main, step_w2)
        return carry

    lax.fori_loop(0, N_UNITS - 1, body, 0)

    j = UNITS - 1
    for a in range(2):
        acc = outacc[a]
        for t in (2 * a, 2 * a + 1):
            lhs = olhs[(2 * t + 1) * 8 + j].astype(BF16)
            view = wo_buf.at[t, 1, pl.ds(j * 128, 128), :]
            pltpu.make_async_copy(view, view, sems.at[3, t]).wait()
            acc = acc + _dot(lhs, view[...], NN)
        out_ref[:, a * 512:(a + 1) * 512] = acc[0:4].astype(out_ref.dtype)


@jax.jit
def pallas_concat_heads__compressed_kv_cla__gqa_block_cached__decode_kernel(
    A_x: jax.Array,
    A_c_kv: jax.Array,
    A_w_q: jax.Array,
    A_w_uk: jax.Array,
    A_w_uv: jax.Array,
    A_w_o: jax.Array,
    B_x: jax.Array,
    B_k_cache: jax.Array,
    B_v_cache: jax.Array,
    B_wq: jax.Array,
    B_wo: jax.Array,
):
    args = (
        A_x.reshape(4, 512),
        A_c_kv.reshape(16, 1024, 512),
        A_w_q.reshape(16384, 128),
        A_w_uk.reshape(16384, 128),
        A_w_uv.reshape(16384, 128),
        A_w_o.reshape(4, 1024, 512),
        B_x.reshape(4, 512),
        B_k_cache.reshape(32, 4096, 128),
        B_v_cache.reshape(32, 4096, 128),
        B_wq.reshape(4, 128, 4096),
        B_wo.reshape(4, 1024, 512),
    )
    vm = pltpu.VMEM
    scratch = [
        vm((4, 512), BF16), vm((4, 512), BF16),
        vm((4, 4096, 128), BF16), vm((4, 4096, 128), BF16), vm((4, 4096, 128), BF16),
        vm((32, 512, 128), BF16), vm((32, 512, 128), BF16), vm((32, 512, 128), BF16),
        vm((4, 128, 4096), BF16),
        vm((4, 2, 1024, 512), BF16),
        vm((8, 4096, 128), BF16),
        vm((2, 1024, 512), BF16),
        vm((2, 8, 512), F32),
        vm((32, 8, 512), F32),
        vm((4, 32, 512), BF16),
        vm((16, 128), BF16),
        vm((16, 1), F32), vm((16, 128), F32), vm((16, 128), F32),
        vm((2, 32, 1), F32), vm((2, 32, 128), F32), vm((2, 32, 512), F32),
        vm((8, 32, 512), F32), vm((32, 8, 512), F32),
        vm((64, 8, 128), F32),
        vm((2, 8, 512), F32),
        pltpu.SemaphoreType.DMA((4, UNITS + 1)),
    ]
    out = pl.pallas_call(
        _kernel,
        out_shape=jax.ShapeDtypeStruct((4, 1024), A_x.dtype),
        in_specs=[pl.BlockSpec(memory_space=pl.ANY)] * 11,
        out_specs=pl.BlockSpec(memory_space=pltpu.VMEM),
        scratch_shapes=scratch,
        compiler_params=pltpu.CompilerParams(
            vmem_limit_bytes=64 * 1024 * 1024,
            disable_bounds_checks=True,
            disable_semaphore_checks=True,
        ),
    )(*args)
    return out.reshape(4, 1, 1024)
```
